```python
import jax
import jax.numpy as jnp

def _softmax(x, axis=-1):
    return jax.nn.softmax(x, axis=axis)
def _gelu(x):
    return jax.nn.gelu(x, approximate=True)
def _silu(x):
    return jax.nn.silu(x)
def _sigmoid(x):
    return jax.nn.sigmoid(x)
def _layernorm(x, axis=-1, eps=1e-5):
    m = jnp.mean(x, axis=axis, keepdims=True)
    v = jnp.var(x, axis=axis, keepdims=True)
    return (x - m) / jnp.sqrt(v + eps)
def _scatter_add(tgt, idx, src, axis=0):
    return tgt.at[idx].add(src)
def _segment_sum(src, seg, n):
    return jax.ops.segment_sum(src, seg, n)
class _Rng:
    def __init__(self, key):
        self._k = key
    def _next(self):
        self._k, sub = jax.random.split(self._k)
        return sub
    def normal(self, shape):
        return jax.random.normal(self._next(), shape, dtype=jnp.bfloat16)
    def randint(self, lo, hi, shape):
        return jax.random.randint(self._next(), shape, lo, hi, dtype=jnp.int32)
    def uniform(self, shape, lo=0.0, hi=1.0):
        return jax.random.uniform(self._next(), shape, jnp.bfloat16, lo, hi)
    def permutation(self, n):
        return jax.random.permutation(self._next(), n)


kernel_name = 'sequential_preLN__sliding_block__glu_gated_glu__prompt'

def _fwd_setup_inputs():
    _rng = _Rng(jax.random.key(int.from_bytes(__import__("os").urandom(4), "little")))
    _w = (lambda a: (lambda t: t.astype(jnp.bfloat16) if jnp.issubdtype(t.dtype, jnp.floating) else t)(jnp.asarray(a)))
    def _A_setup():
        B, S, D = 1, 2048, 512
        return {
            "x": _w((lambda *s: _rng.normal(s) * 0.05)(B, S, D)),
            "wqkv": _w((lambda *s: _rng.normal(s) * 0.05)(D, 3 * D)),
            "wo": _w((lambda *s: _rng.normal(s) * 0.05)(D, D)),
        }
    _A_in = _A_setup()

    def _B_setup():
        B, S, D, F = 1, 2048, 512, 1376
        return {
            "x": _w((lambda *s: _rng.normal(s) * 0.05)(B, S, D)),
            "w_gate": _w((lambda *s: _rng.normal(s) * 0.05)(D, F)),
            "w_up": _w((lambda *s: _rng.normal(s) * 0.05)(D, F)),
            "w_down": _w((lambda *s: _rng.normal(s) * 0.05)(F, D)),
        }
    _B_in = _B_setup()

    return {
        "A_x": _A_in["x"],
        "A_wqkv": _A_in["wqkv"],
        "A_wo": _A_in["wo"],
        "B_x": _B_in["x"],
        "B_w_gate": _B_in["w_gate"],
        "B_w_up": _B_in["w_up"],
        "B_w_down": _B_in["w_down"],
    }

def _fwd_reference(A_x, A_wqkv, A_wo, B_x, B_w_gate, B_w_up, B_w_down):
    def _A_ref(x, wqkv, wo):
        B, S, D = x.shape
        H = 32; Dh = D // H; W = 256
        qkv = (lambda x, *d: x.transpose(*d))((x @ wqkv).reshape(B, S, 3, H, Dh), 2, 0, 3, 1, 4)
        q, k, v = qkv[0], qkv[1], qkv[2]
        scores = jnp.einsum("bhqd,bhkd->bhqk", q, k) * (Dh ** -0.5)
        idx = jnp.arange(S)
        mask = (idx[:, None] - idx[None, :] >= 0) & (idx[:, None] - idx[None, :] < W)
        scores = jnp.where(mask[None, None], scores, -1e9)
        p = _softmax(scores, axis=-1)
        o = jnp.einsum("bhqk,bhkd->bhqd", p, v)
        return (lambda x, *d: x.transpose(*d))(o, 0, 2, 1, 3).reshape(B, S, D) @ wo

    def _B_ref(x, w_gate, w_up, w_down):
        g = jnp.einsum("bsd,df->bsf", x, w_gate)
        u = jnp.einsum("bsd,df->bsf", x, w_up)
        h = _sigmoid(g) * u
        return jnp.einsum("bsf,fd->bsd", h, w_down)

    x = A_x
    h = x + _A_ref(_layernorm(x, axis=-1), A_wqkv, A_wo)
    h2 = h + _B_ref(_layernorm(h, axis=-1), B_w_gate, B_w_up, B_w_down)
    return h2


def setup_inputs():
    _inp = _fwd_setup_inputs()
    _gk = jax.random.fold_in(jax.random.key(int.from_bytes(__import__("os").urandom(4), "little")), 2**31 - 1)
    _shapes = [[1, 2048, 512]]
    _dtypes = ['bfloat16']
    _gks = jax.random.split(_gk, len(_shapes))
    _gs = [jax.random.normal(k, s, dtype=jnp.dtype(d)) * 0.05 for k, s, d in zip(_gks, _shapes, _dtypes)]
    _inp["grad_out"] = _gs[0]
    return _inp

def reference(A_x, A_wqkv, A_wo, B_w_gate, B_w_up, B_w_down, B_x, grad_out):
    _const = dict(B_x=B_x)
    def _f(*_d):
        return _fwd_reference(**{'A_x': _d[0], 'A_wqkv': _d[1], 'A_wo': _d[2], 'B_w_gate': _d[3], 'B_w_up': _d[4], 'B_w_down': _d[5], **_const})
    _out, _vjp = jax.vjp(_f, A_x, A_wqkv, A_wo, B_w_gate, B_w_up, B_w_down)
    _grads = _vjp(grad_out)
    _out0 = jnp.asarray(_out)
    return (_out0, *[jnp.asarray(_g) for _g in _grads])
```

```python
import functools

import jax
import jax.numpy as jnp
from jax import lax
import jax.experimental.pallas as pl
import jax.experimental.pallas.tpu as pltpu

S = 2048
D = 512
F = 1376
H = 32
DH = 16
W = 256
TM = 256
NB = S // TM
QB = 128
NG = 4
KW = 384
PAD = 256
EPS = 1e-5
SCALE = DH ** -0.5
NEG = -1e9

BF = jnp.bfloat16
F32 = jnp.float32

NT = (((1,), (1,)), ((), ()))
TN = (((0,), (0,)), ((), ()))


def _dot(a, b):
    return jnp.dot(a, b, preferred_element_type=F32)


def _dot_nt(a, b):
    return lax.dot_general(a, b, NT, preferred_element_type=F32)


def _dot_tn(a, b):
    return lax.dot_general(a, b, TN, preferred_element_type=F32)


def _ln(x):
    m = jnp.mean(x, axis=-1, keepdims=True)
    xc = x - m
    v = jnp.mean(xc * xc, axis=-1, keepdims=True)
    r = lax.rsqrt(v + EPS)
    return xc * r, r


def _ln_bwd(dy, y, r):
    m1 = jnp.mean(dy, axis=-1, keepdims=True)
    m2 = jnp.mean(dy * y, axis=-1, keepdims=True)
    return (dy - m1 - y * m2) * r


def _kernel(x_ref, xl_ref, dout_ref, wqkv_ref, wo_ref, wg_ref, wu_ref, wd_ref,
            out_ref, dx_ref, dwqkv_ref, dwo_ref, dwg_ref, dwu_ref, dwd_ref,
            q_scr, k_scr, v_scr, kT_scr, vT_scr, pT_scr, oT_scr, do_scr,
            dl_scr, dqT_scr, dk_acc, dv_acc, dq_scr, dh_scr,
            a_wqkv, a_wo, a_wg, a_wu, a_wd):
    i = pl.program_id(0)

    @pl.when(i == 0)
    def _init():
        k_scr[...] = jnp.zeros_like(k_scr)
        v_scr[...] = jnp.zeros_like(v_scr)
        kT_scr[...] = jnp.zeros_like(kT_scr)
        vT_scr[...] = jnp.zeros_like(vT_scr)
        dk_acc[...] = jnp.zeros_like(dk_acc)
        dv_acc[...] = jnp.zeros_like(dv_acc)
        a_wqkv[...] = jnp.zeros_like(a_wqkv)
        a_wo[...] = jnp.zeros_like(a_wo)
        a_wg[...] = jnp.zeros_like(a_wg)
        a_wu[...] = jnp.zeros_like(a_wu)
        a_wd[...] = jnp.zeros_like(a_wd)

    lane = lax.broadcasted_iota(jnp.int32, (QB, 128), 1)
    r_io = lax.broadcasted_iota(jnp.int32, (KW, QB), 0)
    c_io = lax.broadcasted_iota(jnp.int32, (KW, QB), 1)
    band = (r_io > c_io) & (r_io <= c_io + W)

    @pl.when(i < NB)
    def _main():
        slot = i % 2
        x = x_ref[...].astype(F32)
        xn, _ = _ln(x)
        xn_b = xn.astype(BF)
        qkv = _dot(xn_b, wqkv_ref[...])
        row0 = pl.multiple_of(PAD + i * TM, TM)
        for g in range(NG):
            q_scr[g] = (qkv[:, g * 128:(g + 1) * 128] * SCALE).astype(BF)
            kk = qkv[:, D + g * 128:D + (g + 1) * 128]
            vv = qkv[:, 2 * D + g * 128:2 * D + (g + 1) * 128]
            k_scr[g, pl.ds(row0, TM), :] = kk.astype(BF)
            v_scr[g, pl.ds(row0, TM), :] = vv.astype(BF)
            kkT = kk.T.astype(BF)
            vvT = vv.T.astype(BF)
            for b in range(2):
                kT_scr[g, 2 + 2 * i + b] = kkT[:, b * 128:(b + 1) * 128]
                vT_scr[g, 2 + 2 * i + b] = vvT[:, b * 128:(b + 1) * 128]

        def fwd_body(t, carry):
            b = t // NG
            g = t % NG
            B = 2 * i + b
            krow = pl.multiple_of(B * QB, QB)
            mask = band & (r_io >= PAD - B * QB)
            qg = q_scr[g, pl.ds(pl.multiple_of(b * QB, QB), QB), :]
            kg = k_scr[g, pl.ds(krow, KW), :]
            for hh in range(8):
                qm = jnp.where(lane // DH == hh, qg, jnp.zeros_like(qg))
                sT = _dot_nt(kg, qm)
                sT = jnp.where(mask, sT, NEG)
                m = jnp.max(sT, axis=0, keepdims=True)
                e = jnp.exp(sT - m)
                l = jnp.sum(e, axis=0, keepdims=True)
                pT = (e * (1.0 / l)).astype(BF)
                pT_scr[t * 8 + hh] = pT
                oT = None
                for kb in range(3):
                    vt = vT_scr[g, B + kb, hh * DH:(hh + 1) * DH, :]
                    c = _dot(vt, pT[kb * 128:(kb + 1) * 128, :])
                    oT = c if oT is None else oT + c
                oT_scr[b, pl.ds(pl.multiple_of(g * 128 + hh * DH, DH), DH), :] = oT
            return carry

        lax.fori_loop(0, 2 * NG, fwd_body, 0)

        oT = jnp.concatenate([oT_scr[0], oT_scr[1]], axis=1)
        o = oT.T
        o_b = o.astype(BF)
        h = x + _dot(o_b, wo_ref[...])
        hn, r2 = _ln(h)
        hn_b = hn.astype(BF)
        gt = _dot(hn_b, wg_ref[...])
        up = _dot(hn_b, wu_ref[...])
        sg = jax.nn.sigmoid(gt)
        a_b = (sg * up).astype(BF)
        out = h + _dot(a_b, wd_ref[...])
        out_ref[...] = out.astype(out_ref.dtype)

        dout_b = dout_ref[...]
        dout = dout_b.astype(F32)
        da = _dot_nt(dout_b, wd_ref[...])
        a_wd[...] += _dot_tn(a_b, dout_b)
        du_b = (da * sg).astype(BF)
        dg_b = (da * up * sg * (1.0 - sg)).astype(BF)
        a_wg[...] += _dot_tn(hn_b, dg_b)
        a_wu[...] += _dot_tn(hn_b, du_b)
        dhn = _dot_nt(dg_b, wg_ref[...]) + _dot_nt(du_b, wu_ref[...])
        dh = dout + _ln_bwd(dhn, hn, r2)
        dh_scr[slot] = dh
        dh_b = dh.astype(BF)
        a_wo[...] += _dot_tn(o_b, dh_b)
        do = _dot_nt(dh_b, wo_ref[...])
        for g in range(NG):
            do_scr[g] = do[:, g * 128:(g + 1) * 128].astype(BF)
        prod = do.T * oT
        dl = jnp.sum(prod.reshape(H, DH, TM), axis=1)
        dl_scr[0] = dl[:, 0:128]
        dl_scr[1] = dl[:, 128:256]

        def bwd_body(t, carry):
            b = t // NG
            g = t % NG
            B = 2 * i + b
            krow = pl.multiple_of(B * QB, QB)
            qrow = pl.multiple_of(b * QB, QB)
            qg = q_scr[g, pl.ds(qrow, QB), :]
            dog = do_scr[g, pl.ds(qrow, QB), :]
            kg = k_scr[g, pl.ds(krow, KW), :]
            vg = v_scr[g, pl.ds(krow, KW), :]
            dk = None
            dv = None
            for hh in range(8):
                hm = lane // DH == hh
                qm = jnp.where(hm, qg, jnp.zeros_like(qg))
                dom = jnp.where(hm, dog, jnp.zeros_like(dog))
                dpT = _dot_nt(vg, dom)
                pT = pT_scr[t * 8 + hh]
                delta = dl_scr[b, pl.ds(g * 8 + hh, 1), :]
                dsT = (pT.astype(F32) * (dpT - delta)).astype(BF)
                c1 = _dot(pT, dom)
                c2 = _dot(dsT, qm)
                dv = c1 if dv is None else dv + c1
                dk = c2 if dk is None else dk + c2
                dqT = None
                for kb in range(3):
                    kt = kT_scr[g, B + kb, hh * DH:(hh + 1) * DH, :]
                    c = _dot(kt, dsT[kb * 128:(kb + 1) * 128, :])
                    dqT = c if dqT is None else dqT + c
                dqT_scr[b, pl.ds(pl.multiple_of(g * 128 + hh * DH, DH), DH), :] = dqT * SCALE
            dk_acc[g, pl.ds(krow, KW), :] += dk
            dv_acc[g, pl.ds(krow, KW), :] += dv
            return carry

        lax.fori_loop(0, 2 * NG, bwd_body, 0)
        dqT = jnp.concatenate([dqT_scr[0], dqT_scr[1]], axis=1)
        dq_scr[slot] = dqT.T

    @pl.when(i > 0)
    def _lag():
        j = i - 1
        slot = j % 2
        xl = xl_ref[...].astype(F32)
        xn, r1 = _ln(xl)
        xn_b = xn.astype(BF)
        row0 = pl.multiple_of(PAD + j * TM, TM)
        parts = [dq_scr[slot].astype(BF)]
        for g in range(NG):
            parts.append(dk_acc[g, pl.ds(row0, TM), :].astype(BF))
        for g in range(NG):
            parts.append(dv_acc[g, pl.ds(row0, TM), :].astype(BF))
        dqkv_b = jnp.concatenate(parts, axis=1)
        a_wqkv[...] += _dot_tn(xn_b, dqkv_b)
        dxn = _dot_nt(dqkv_b, wqkv_ref[...])
        dx = dh_scr[slot] + _ln_bwd(dxn, xn, r1)
        dx_ref[...] = dx.astype(dx_ref.dtype)

    @pl.when(i == NB)
    def _fin():
        dwqkv_ref[...] = a_wqkv[...].astype(BF)
        dwo_ref[...] = a_wo[...].astype(BF)
        dwg_ref[...] = a_wg[...].astype(BF)
        dwu_ref[...] = a_wu[...].astype(BF)
        dwd_ref[...] = a_wd[...].astype(BF)


@jax.jit
def pallas_sequential_preLN__sliding_block__glu_gated_glu__prompt_kernel(
    A_x: jax.Array,
    A_wqkv: jax.Array,
    A_wo: jax.Array,
    B_x: jax.Array,
    B_w_gate: jax.Array,
    B_w_up: jax.Array,
    B_w_down: jax.Array,
    grad_out: jax.Array,
):
    x2 = A_x.reshape(S, D)
    go = grad_out.reshape(S, D)

    cur = lambda i: (jnp.minimum(i, NB - 1), 0)
    lag = lambda i: (jnp.maximum(i - 1, 0), 0)
    const = lambda i: (0, 0)
    NKB = (PAD + S) // 128

    out_shape = (
        jax.ShapeDtypeStruct((S, D), BF),
        jax.ShapeDtypeStruct((S, D), BF),
        jax.ShapeDtypeStruct((D, 3 * D), BF),
        jax.ShapeDtypeStruct((D, D), BF),
        jax.ShapeDtypeStruct((D, F), BF),
        jax.ShapeDtypeStruct((D, F), BF),
        jax.ShapeDtypeStruct((F, D), BF),
    )
    in_specs = [
        pl.BlockSpec((TM, D), cur),
        pl.BlockSpec((TM, D), lag),
        pl.BlockSpec((TM, D), cur),
        pl.BlockSpec((D, 3 * D), const),
        pl.BlockSpec((D, D), const),
        pl.BlockSpec((D, F), const),
        pl.BlockSpec((D, F), const),
        pl.BlockSpec((F, D), const),
    ]
    out_specs = (
        pl.BlockSpec((TM, D), cur),
        pl.BlockSpec((TM, D), lag),
        pl.BlockSpec((D, 3 * D), const),
        pl.BlockSpec((D, D), const),
        pl.BlockSpec((D, F), const),
        pl.BlockSpec((D, F), const),
        pl.BlockSpec((F, D), const),
    )
    scratch = [
        pltpu.VMEM((NG, TM, 128), BF),
        pltpu.VMEM((NG, PAD + S, 128), BF),
        pltpu.VMEM((NG, PAD + S, 128), BF),
        pltpu.VMEM((NG, NKB, 128, 128), BF),
        pltpu.VMEM((NG, NKB, 128, 128), BF),
        pltpu.VMEM((2 * H, KW, QB), BF),
        pltpu.VMEM((2, D, QB), F32),
        pltpu.VMEM((NG, TM, 128), BF),
        pltpu.VMEM((2, H, QB), F32),
        pltpu.VMEM((2, D, QB), F32),
        pltpu.VMEM((NG, PAD + S, 128), F32),
        pltpu.VMEM((NG, PAD + S, 128), F32),
        pltpu.VMEM((2, TM, D), F32),
        pltpu.VMEM((2, TM, D), F32),
        pltpu.VMEM((D, 3 * D), F32),
        pltpu.VMEM((D, D), F32),
        pltpu.VMEM((D, F), F32),
        pltpu.VMEM((D, F), F32),
        pltpu.VMEM((F, D), F32),
    ]
    outs = pl.pallas_call(
        _kernel,
        grid=(NB + 1,),
        in_specs=in_specs,
        out_specs=out_specs,
        out_shape=out_shape,
        scratch_shapes=scratch,
        compiler_params=pltpu.CompilerParams(
            dimension_semantics=("arbitrary",),
            vmem_limit_bytes=100 * 1024 * 1024,
        ),
    )(x2, x2, go, A_wqkv, A_wo, B_w_gate, B_w_up, B_w_down)
    fwd, dx, dwqkv, dwo, dwg, dwu, dwd = outs
    return (fwd.reshape(1, S, D), dx.reshape(1, S, D), dwqkv, dwo, dwg, dwu, dwd)
```

```python
import contextlib
import functools
import os

import jax
import jax.numpy as jnp
from jax import lax
import jax.experimental.pallas as pl
import jax.experimental.pallas.tpu as pltpu

S = 2048
D = 512
F = 1376
H = 32
DH = 16
W = 256
TM = 256
NB = S // TM
QB = 128
NG = 4
HG = 8
KW = 384
PAD = 256
NKB = (PAD + S) // 128
EPS = 1e-5
SCALE = DH ** -0.5
LOG2E = 1.4426950408889634
NEG = -1e9

BF = jnp.bfloat16
F32 = jnp.float32

_PROF = os.environ.get('KPROF', '0') == '1'


def _scope(name):
    return jax.named_scope(name) if _PROF else contextlib.nullcontext()


NT = (((1,), (1,)), ((), ()))
TN = (((0,), (0,)), ((), ()))


def _dot(a, b):
    return jnp.dot(a, b, preferred_element_type=F32)


def _dot_nt(a, b):
    return lax.dot_general(a, b, NT, preferred_element_type=F32)


def _dot_tn(a, b):
    return lax.dot_general(a, b, TN, preferred_element_type=F32)


def _ln(x):
    m = jnp.mean(x, axis=-1, keepdims=True)
    xc = x - m
    v = jnp.mean(xc * xc, axis=-1, keepdims=True)
    r = lax.rsqrt(v + EPS)
    return xc * r, r


def _ln_bwd(dy, y, r):
    m1 = jnp.mean(dy, axis=-1, keepdims=True)
    m2 = jnp.mean(dy * y, axis=-1, keepdims=True)
    return (dy - m1 - y * m2) * r


def _colred(x, op):
    n = x.shape[0]
    while n > 8:
        n //= 2
        x = op(x[:n], x[n:])
    if op is jnp.maximum:
        return jnp.max(x, axis=0, keepdims=True)
    return jnp.sum(x, axis=0, keepdims=True)


def _kernel(x_ref, xl_ref, dout_ref, wqkv_hbm, wo_hbm, wg_hbm, wu_hbm, wd_hbm,
            out_ref, dx_ref, dwqkv_hbm, dwo_hbm, dwg_hbm, dwu_hbm, dwd_hbm,
            q_scr, qT_scr, kn_scr, vn_scr, kT_scr, vT_scr, eT_scr, f_scr, oT_scr,
            do_scr, doT_scr, dl_scr, dqT_scr, dkT_acc, dvT_acc, dh_scr,
            a_wqkv, a_wo, a_wg, a_wu, a_wd, bd_scr, s_scr, ds_scr,
            wqkv_ref, wo_ref, wg_ref, wu_ref, wd_ref,
            o_wqkv, o_wo, o_wg, o_wu, o_wd, sem):
    i = pl.program_id(0)

    def w_copy(k):
        srcs = (wqkv_hbm, wo_hbm, wg_hbm, wu_hbm, wd_hbm)
        dsts = (wqkv_ref, wo_ref, wg_ref, wu_ref, wd_ref)
        return pltpu.make_async_copy(srcs[k], dsts[k], sem.at[k])

    def g_copy(k):
        srcs = (o_wqkv, o_wo, o_wg, o_wu, o_wd)
        dsts = (dwqkv_hbm, dwo_hbm, dwg_hbm, dwu_hbm, dwd_hbm)
        return pltpu.make_async_copy(srcs[k], dsts[k], sem.at[5 + k])

    @pl.when(i == 0)
    def _init():
        with _scope('init'):
            for k in range(5):
                w_copy(k).start()
            zb = jnp.zeros((PAD, 128), BF)
            zf = jnp.zeros((128, 128), F32)
            row = lax.broadcasted_iota(jnp.int32, vT_scr.shape[1:], 2)
            ones_rows = jnp.where(row >= DH, 1.0, 0.0).astype(BF)
            for g in range(NG):
                kn_scr[g, 0:PAD, :] = zb
                vn_scr[g, 0:PAD, :] = zb
                vT_scr[g] = ones_rows
                for blk in range(2):
                    kT_scr[g, blk] = zf.astype(BF)
                    dkT_acc[g, blk] = zf
                    dvT_acc[g, blk] = zf
            a_wqkv[...] = jnp.zeros_like(a_wqkv)
            a_wo[...] = jnp.zeros_like(a_wo)
            a_wg[...] = jnp.zeros_like(a_wg)
            a_wu[...] = jnp.zeros_like(a_wu)
            a_wd[...] = jnp.zeros_like(a_wd)
            w_copy(0).wait()

    lane64 = lax.broadcasted_iota(jnp.int32, (QB // 2, 128), 1)
    r_io = lax.broadcasted_iota(jnp.int32, (128, QB), 0)
    c_io = lax.broadcasted_iota(jnp.int32, (128, QB), 1)
    mask0 = r_io > c_io
    mask2 = r_io <= c_io

    @pl.when(i < NB)
    def _main():
        slot = i % 2
        with _scope('qkv'):
            x = x_ref[...].astype(F32)
            xn, _ = _ln(x)
            xn_b = xn.astype(BF)
            qkv = _dot(xn_b, wqkv_ref[...])
            row0 = pl.multiple_of(PAD + i * TM, TM)
            for g in range(NG):
                qq = qkv[:, g * 128:(g + 1) * 128] * (SCALE * LOG2E)
                kk = qkv[:, D + g * 128:D + (g + 1) * 128]
                vv = qkv[:, 2 * D + g * 128:2 * D + (g + 1) * 128]
                q_scr[g] = qq.astype(BF)
                kn_scr[g, pl.ds(row0, TM), :] = kk.astype(BF)
                vn_scr[g, pl.ds(row0, TM), :] = vv.astype(BF)
                qqT = qq.T.astype(BF)
                kkT = kk.T.astype(BF)
                vvT = vv.T.astype(BF)
                for b in range(2):
                    qT_scr[b, g * 128:(g + 1) * 128, :] = qqT[:, b * 128:(b + 1) * 128]
                    kT_scr[g, 2 + 2 * i + b] = kkT[:, b * 128:(b + 1) * 128]
                    for hh in range(HG):
                        vT_scr[g, 2 + 2 * i + b, hh, 0:DH, :] = vvT[hh * DH:(hh + 1) * DH, b * 128:(b + 1) * 128]

        def fwd_body(t, carry):
            b = t // NG
            g = t % NG
            B = 2 * i + b
            qg = q_scr[g, pl.ds(pl.multiple_of(b * QB, QB), QB), :]
            qi = pltpu.bitcast(qg, jnp.int32)
            for hh in range(HG):
                bd_scr[hh * 128:(hh + 1) * 128, :] = pltpu.bitcast(
                    jnp.where(lane64 // DH == hh, qi, jnp.zeros_like(qi)), BF)
            kwin = kn_scr[g, pl.ds(pl.multiple_of(B * 128, 128), KW), :]
            s_scr[...] = _dot_nt(kwin, bd_scr[...])
            ms = []
            for hh in range(HG):
                mh = []
                for kb in range(3):
                    s = s_scr[kb * 128:(kb + 1) * 128, hh * 128:(hh + 1) * 128]
                    if kb == 0:
                        s = jnp.where(mask0, s, NEG)
                    elif kb == 2:
                        s = jnp.where(mask2, s, NEG)
                    m = _colred(s, jnp.maximum)
                    eT_scr[t * HG + hh, kb * 128:(kb + 1) * 128, :] = jnp.exp2(s - m).astype(BF)
                    mh.append(m)
                ms.append(mh)
            for hh in range(HG):
                ols = []
                for kb in range(3):
                    ols.append(_dot(vT_scr[g, B + kb, hh], eT_scr[t * HG + hh, kb * 128:(kb + 1) * 128, :]))
                m0 = jnp.where(B >= 2, ms[hh][0], NEG)
                m1 = jnp.where(B >= 1, ms[hh][1], NEG)
                m2 = ms[hh][2]
                mm = jnp.maximum(jnp.maximum(m0, m1), m2)
                c0 = jnp.where(B >= 2, jnp.exp2(m0 - mm), 0.0)
                c1 = jnp.where(B >= 1, jnp.exp2(m1 - mm), 0.0)
                c2 = jnp.exp2(m2 - mm)
                l = c0 * ols[0][DH:DH + 1] + c1 * ols[1][DH:DH + 1] + c2 * ols[2][DH:DH + 1]
                rl = 1.0 / l
                f0 = c0 * rl
                f1 = c1 * rl
                f2 = c2 * rl
                oT = ols[0][:DH] * f0 + ols[1][:DH] * f1 + ols[2][:DH] * f2
                oT_scr[b, pl.ds(pl.multiple_of(g * 128 + hh * DH, DH), DH), :] = oT
                f_scr[t * HG + hh, 0:1, :] = f0
                f_scr[t * HG + hh, 1:2, :] = f1
                f_scr[t * HG + hh, 2:3, :] = f2
            return carry

        with _scope('attn_fwd'):
            lax.fori_loop(0, 2 * NG, fwd_body, 0)

        @pl.when(i == 0)
        def _wait_w():
            for k in range(1, 5):
                w_copy(k).wait()

        with _scope('mlp_fwd'):
            oT = jnp.concatenate([oT_scr[0], oT_scr[1]], axis=1)
            o = oT.T
            o_b = o.astype(BF)
            h = x + _dot(o_b, wo_ref[...])
            hn, r2 = _ln(h)
            hn_b = hn.astype(BF)
            gt = _dot_nt(hn_b, wg_ref[...])
            up = _dot_nt(hn_b, wu_ref[...])
            sg = jax.nn.sigmoid(gt)
            a_b = (sg * up).astype(BF)
            out = h + _dot(a_b, wd_ref[...])
            out_ref[...] = out.astype(out_ref.dtype)

        with _scope('mlp_bwd'):
            dout_b = dout_ref[...]
            dout = dout_b.astype(F32)
            da = _dot_nt(dout_b, wd_ref[...])
            a_wd[...] += _dot_tn(a_b, dout_b)
            du_b = (da * sg).astype(BF)
            dg_b = (da * up * sg * (1.0 - sg)).astype(BF)
            a_wg[...] += _dot_tn(dg_b, hn_b)
            a_wu[...] += _dot_tn(du_b, hn_b)
            dhn = _dot(dg_b, wg_ref[...]) + _dot(du_b, wu_ref[...])
            dh = dout + _ln_bwd(dhn, hn, r2)
            dh_scr[slot] = dh
        with _scope('wo_bwd'):
            dh_b = dh.astype(BF)
            a_wo[...] += _dot_tn(o_b, dh_b)
            do = _dot_nt(dh_b, wo_ref[...])
            for g in range(NG):
                do_scr[g] = do[:, g * 128:(g + 1) * 128].astype(BF)
            doT = do.T
            doT_scr[0] = doT[:, 0:128]
            doT_scr[1] = doT[:, 128:256]
            prod = doT * oT
            dl = jnp.sum(prod.reshape(H, DH, TM), axis=1)
            dl_scr[0] = dl[:, 0:128]
            dl_scr[1] = dl[:, 128:256]

        @pl.when(i == NB - 1)
        def _flush_mlp():
            o_wd[...] = a_wd[...].astype(BF)
            g_copy(4).start()
            o_wg[...] = a_wg[...].astype(BF)
            g_copy(2).start()
            o_wu[...] = a_wu[...].astype(BF)
            g_copy(3).start()
            o_wo[...] = a_wo[...].astype(BF)
            g_copy(1).start()

        def bwd_body(t, carry):
            b = t // NG
            g = t % NG
            B = 2 * i + b
            dog = do_scr[g, pl.ds(pl.multiple_of(b * QB, QB), QB), :]
            di = pltpu.bitcast(dog, jnp.int32)
            for hh in range(HG):
                bd_scr[hh * 128:(hh + 1) * 128, :] = pltpu.bitcast(
                    jnp.where(lane64 // DH == hh, di, jnp.zeros_like(di)), BF)
            vwin = vn_scr[g, pl.ds(pl.multiple_of(B * 128, 128), KW), :]
            s_scr[...] = _dot_nt(vwin, bd_scr[...])
            for hh in range(HG):
                delta = dl_scr[b, pl.ds(g * HG + hh, 1), :]
                for kb in range(3):
                    dp = s_scr[kb * 128:(kb + 1) * 128, hh * 128:(hh + 1) * 128]
                    e = eT_scr[t * HG + hh, kb * 128:(kb + 1) * 128, :]
                    f = f_scr[t * HG + hh, kb:kb + 1, :]
                    ds_scr[hh, kb * 128:(kb + 1) * 128, :] = (e.astype(F32) * ((dp - delta) * f)).astype(BF)
            for hh in range(HG):
                hrow = pl.multiple_of(g * 128 + hh * DH, DH)
                doT_h = doT_scr[b, pl.ds(hrow, DH), :]
                qT_h = qT_scr[b, pl.ds(hrow, DH), :]
                dqT = None
                for kb in range(3):
                    e = eT_scr[t * HG + hh, kb * 128:(kb + 1) * 128, :]
                    ds = ds_scr[hh, kb * 128:(kb + 1) * 128, :]
                    f = f_scr[t * HG + hh, kb:kb + 1, :]
                    cv = _dot_nt((doT_h * f).astype(BF), e)
                    ck = _dot_nt(qT_h, ds)
                    if kb == 2:
                        dvT_acc[g, B + kb, hh * DH:(hh + 1) * DH, :] = cv
                        dkT_acc[g, B + kb, hh * DH:(hh + 1) * DH, :] = ck
                    else:
                        dvT_acc[g, B + kb, hh * DH:(hh + 1) * DH, :] += cv
                        dkT_acc[g, B + kb, hh * DH:(hh + 1) * DH, :] += ck
                    c = _dot(kT_scr[g, B + kb, hh * DH:(hh + 1) * DH, :], ds)
                    dqT = c if dqT is None else dqT + c
                dqT_scr[slot, b, pl.ds(hrow, DH), :] = dqT * SCALE
            return carry

        with _scope('attn_bwd'):
            lax.fori_loop(0, 2 * NG, bwd_body, 0)

    @pl.when(i > 0)
    def _lag():
        with _scope('lag'):
            j = i - 1
            slot = j % 2
            xl = xl_ref[...].astype(F32)
            xn, r1 = _ln(xl)
            xnT_b = xn.T.astype(BF)
            cols = []
            for b in range(2):
                parts = [dqT_scr[slot, b].astype(BF)]
                for g in range(NG):
                    parts.append((dkT_acc[g, 2 + 2 * j + b] * (1.0 / LOG2E)).astype(BF))
                for g in range(NG):
                    parts.append(dvT_acc[g, 2 + 2 * j + b].astype(BF))
                cols.append(jnp.concatenate(parts, axis=0))
            dqkvT_b = jnp.concatenate(cols, axis=1)
            a_wqkv[...] += _dot_nt(xnT_b, dqkvT_b)
            dxn = _dot(wqkv_ref[...], dqkvT_b).T
            dx = dh_scr[slot] + _ln_bwd(dxn, xn, r1)
            dx_ref[...] = dx.astype(dx_ref.dtype)

    @pl.when(i == NB)
    def _fin():
        o_wqkv[...] = a_wqkv[...].astype(BF)
        g_copy(0).start()
        for k in (4, 2, 3, 1, 0):
            g_copy(k).wait()


@jax.jit
def pallas_sequential_preLN__sliding_block__glu_gated_glu__prompt_kernel(
    A_x: jax.Array,
    A_wqkv: jax.Array,
    A_wo: jax.Array,
    B_x: jax.Array,
    B_w_gate: jax.Array,
    B_w_up: jax.Array,
    B_w_down: jax.Array,
    grad_out: jax.Array,
):
    x2 = A_x.reshape(S, D)
    go = grad_out.reshape(S, D)

    cur = lambda i: (jnp.minimum(i, NB - 1), 0)
    lag = lambda i: (jnp.maximum(i - 1, 0), 0)
    const = lambda i: (0, 0)

    out_shape = (
        jax.ShapeDtypeStruct((S, D), BF),
        jax.ShapeDtypeStruct((S, D), BF),
        jax.ShapeDtypeStruct((D, 3 * D), BF),
        jax.ShapeDtypeStruct((D, D), BF),
        jax.ShapeDtypeStruct((F, D), BF),
        jax.ShapeDtypeStruct((F, D), BF),
        jax.ShapeDtypeStruct((F, D), BF),
    )
    in_specs = [
        pl.BlockSpec((TM, D), cur),
        pl.BlockSpec((TM, D), lag),
        pl.BlockSpec((TM, D), cur),
        pl.BlockSpec(memory_space=pl.ANY),
        pl.BlockSpec(memory_space=pl.ANY),
        pl.BlockSpec(memory_space=pl.ANY),
        pl.BlockSpec(memory_space=pl.ANY),
        pl.BlockSpec(memory_space=pl.ANY),
    ]
    out_specs = (
        pl.BlockSpec((TM, D), cur),
        pl.BlockSpec((TM, D), lag),
        pl.BlockSpec(memory_space=pl.ANY),
        pl.BlockSpec(memory_space=pl.ANY),
        pl.BlockSpec(memory_space=pl.ANY),
        pl.BlockSpec(memory_space=pl.ANY),
        pl.BlockSpec(memory_space=pl.ANY),
    )
    scratch = [
        pltpu.VMEM((NG, TM, 128), BF),
        pltpu.VMEM((2, D, QB), BF),
        pltpu.VMEM((NG, PAD + S, 128), BF),
        pltpu.VMEM((NG, PAD + S, 128), BF),
        pltpu.VMEM((NG, NKB, 128, 128), BF),
        pltpu.VMEM((NG, NKB, HG, 32, 128), BF),
        pltpu.VMEM((2 * H, KW, QB), BF),
        pltpu.VMEM((2 * H, 8, QB), F32),
        pltpu.VMEM((2, D, QB), F32),
        pltpu.VMEM((NG, TM, 128), BF),
        pltpu.VMEM((2, D, QB), F32),
        pltpu.VMEM((2, H, QB), F32),
        pltpu.VMEM((2, 2, D, QB), F32),
        pltpu.VMEM((NG, NKB, 128, 128), F32),
        pltpu.VMEM((NG, NKB, 128, 128), F32),
        pltpu.VMEM((2, TM, D), F32),
        pltpu.VMEM((D, 3 * D), F32),
        pltpu.VMEM((D, D), F32),
        pltpu.VMEM((F, D), F32),
        pltpu.VMEM((F, D), F32),
        pltpu.VMEM((F, D), F32),
        pltpu.VMEM((HG * 128, 128), BF),
        pltpu.VMEM((KW, HG * 128), F32),
        pltpu.VMEM((HG, KW, 128), BF),
        pltpu.VMEM((D, 3 * D), BF),
        pltpu.VMEM((D, D), BF),
        pltpu.VMEM((F, D), BF),
        pltpu.VMEM((F, D), BF),
        pltpu.VMEM((F, D), BF),
        pltpu.VMEM((D, 3 * D), BF),
        pltpu.VMEM((D, D), BF),
        pltpu.VMEM((F, D), BF),
        pltpu.VMEM((F, D), BF),
        pltpu.VMEM((F, D), BF),
        pltpu.SemaphoreType.DMA((10,)),
    ]
    outs = pl.pallas_call(
        _kernel,
        grid=(NB + 1,),
        in_specs=in_specs,
        out_specs=out_specs,
        out_shape=out_shape,
        scratch_shapes=scratch,
        compiler_params=pltpu.CompilerParams(
            dimension_semantics=("arbitrary",),
            vmem_limit_bytes=100 * 1024 * 1024,
        ),
    )(x2, x2, go, A_wqkv, A_wo, B_w_gate.T, B_w_up.T, B_w_down)
    fwd, dx, dwqkv, dwo, dwg, dwu, dwd = outs
    return (fwd.reshape(1, S, D), dx.reshape(1, S, D), dwqkv, dwo, dwg.T, dwu.T, dwd)
```

```python
import jax
import jax.numpy as jnp
from jax import lax
import jax.experimental.pallas as pl
import jax.experimental.pallas.tpu as pltpu

S = 2048
D = 512
F = 1376
H = 32
DH = 16
W = 256
TM = 256
NB = S // TM
QB = 128
NG = 4
HG = 8
KW = 384
PAD = 256
NKB = (PAD + S) // 128
EPS = 1e-5
SCALE = DH ** -0.5
LOG2E = 1.4426950408889634
NEG = -1e9

BF = jnp.bfloat16
F32 = jnp.float32

NT = (((1,), (1,)), ((), ()))
TN = (((0,), (0,)), ((), ()))


def _dot(a, b):
    return jnp.dot(a, b, preferred_element_type=F32)


def _dot_nt(a, b):
    return lax.dot_general(a, b, NT, preferred_element_type=F32)


def _dot_tn(a, b):
    return lax.dot_general(a, b, TN, preferred_element_type=F32)


def _ln(x):
    m = jnp.mean(x, axis=-1, keepdims=True)
    xc = x - m
    v = jnp.mean(xc * xc, axis=-1, keepdims=True)
    r = lax.rsqrt(v + EPS)
    return xc * r, r


def _ln_bwd(dy, y, r):
    m1 = jnp.mean(dy, axis=-1, keepdims=True)
    m2 = jnp.mean(dy * y, axis=-1, keepdims=True)
    return (dy - m1 - y * m2) * r


def _colred(x, op):
    n = x.shape[0]
    while n > 8:
        n //= 2
        x = op(x[:n], x[n:])
    if op is jnp.maximum:
        return jnp.max(x, axis=0, keepdims=True)
    return jnp.sum(x, axis=0, keepdims=True)


def _kernel(x_ref, xl_ref, dout_ref, wqkv_hbm, wo_hbm, wg_hbm, wu_hbm, wd_hbm,
            out_ref, dx_ref, dwqkv_hbm, dwo_hbm, dwg_hbm, dwu_hbm, dwd_hbm,
            q_scr, qT_scr, kn_scr, vn_scr, kT_scr, vT_scr, eT_scr, f_scr, oT_scr,
            do_scr, doT_scr, dl_scr, dqT_scr, dkT_acc, dvT_acc, dh_scr,
            a_wqkv, a_wo, a_wg, a_wu, a_wd, bd_scr, s_scr, ds_scr,
            wqkv_ref, wo_ref, wg_ref, wu_ref, wd_ref,
            o_wqkv, o_wo, o_wg, o_wu, o_wd, sem):
    i = pl.program_id(0)

    def w_copy(k):
        srcs = (wqkv_hbm, wo_hbm, wg_hbm, wu_hbm, wd_hbm)
        dsts = (wqkv_ref, wo_ref, wg_ref, wu_ref, wd_ref)
        return pltpu.make_async_copy(srcs[k], dsts[k], sem.at[k])

    def g_copy(k):
        srcs = (o_wqkv, o_wo, o_wg, o_wu, o_wd)
        dsts = (dwqkv_hbm, dwo_hbm, dwg_hbm, dwu_hbm, dwd_hbm)
        return pltpu.make_async_copy(srcs[k], dsts[k], sem.at[5 + k])

    @pl.when(i == 0)
    def _init():
        for k in range(5):
            w_copy(k).start()
        zb = jnp.zeros((PAD, 128), BF)
        zf = jnp.zeros((128, 128), F32)
        row = lax.broadcasted_iota(jnp.int32, vT_scr.shape[1:], 2)
        ones_rows = jnp.where(row >= DH, 1.0, 0.0).astype(BF)
        for g in range(NG):
            kn_scr[g, 0:PAD, :] = zb
            vn_scr[g, 0:PAD, :] = zb
            vT_scr[g] = ones_rows
            for blk in range(2):
                kT_scr[g, blk] = zf.astype(BF)
                dkT_acc[g, blk] = zf
                dvT_acc[g, blk] = zf
        a_wqkv[...] = jnp.zeros_like(a_wqkv)
        a_wo[...] = jnp.zeros_like(a_wo)
        a_wg[...] = jnp.zeros_like(a_wg)
        a_wu[...] = jnp.zeros_like(a_wu)
        a_wd[...] = jnp.zeros_like(a_wd)
        w_copy(0).wait()

    lane64 = lax.broadcasted_iota(jnp.int32, (QB // 2, 128), 1)
    r_io = lax.broadcasted_iota(jnp.int32, (128, QB), 0)
    c_io = lax.broadcasted_iota(jnp.int32, (128, QB), 1)
    mask0 = r_io > c_io
    mask2 = r_io <= c_io

    @pl.when(i < NB)
    def _main():
        slot = i % 2
        x = x_ref[...].astype(F32)
        xn, _ = _ln(x)
        xn_b = xn.astype(BF)
        qkv = _dot(xn_b, wqkv_ref[...])
        row0 = pl.multiple_of(PAD + i * TM, TM)
        for g in range(NG):
            qq = qkv[:, g * 128:(g + 1) * 128] * (SCALE * LOG2E)
            kk = qkv[:, D + g * 128:D + (g + 1) * 128]
            vv = qkv[:, 2 * D + g * 128:2 * D + (g + 1) * 128]
            q_scr[g] = qq.astype(BF)
            kn_scr[g, pl.ds(row0, TM), :] = kk.astype(BF)
            vn_scr[g, pl.ds(row0, TM), :] = vv.astype(BF)
            qqT = qq.T.astype(BF)
            kkT = kk.T.astype(BF)
            vvT = vv.T.astype(BF)
            for b in range(2):
                qT_scr[b, g * 128:(g + 1) * 128, :] = qqT[:, b * 128:(b + 1) * 128]
                kT_scr[g, 2 + 2 * i + b] = kkT[:, b * 128:(b + 1) * 128]
                for hh in range(HG):
                    vT_scr[g, 2 + 2 * i + b, hh, 0:DH, :] = vvT[hh * DH:(hh + 1) * DH, b * 128:(b + 1) * 128]

        def fwd_body(t, carry):
            b = t // NG
            g = t % NG
            B = 2 * i + b
            qg = q_scr[g, pl.ds(pl.multiple_of(b * QB, QB), QB), :]
            qi = pltpu.bitcast(qg, jnp.int32)
            for hh in range(HG):
                bd_scr[hh * 128:(hh + 1) * 128, :] = pltpu.bitcast(
                    jnp.where(lane64 // DH == hh, qi, jnp.zeros_like(qi)), BF)
            kwin = kn_scr[g, pl.ds(pl.multiple_of(B * 128, 128), KW), :]
            s_scr[...] = _dot_nt(kwin, bd_scr[...])
            ms = []
            for hh in range(HG):
                mh = []
                for kb in range(3):
                    s = s_scr[kb * 128:(kb + 1) * 128, hh * 128:(hh + 1) * 128]
                    if kb == 0:
                        s = jnp.where(mask0, s, NEG)
                    elif kb == 2:
                        s = jnp.where(mask2, s, NEG)
                    m = _colred(s, jnp.maximum)
                    eT_scr[t * HG + hh, kb * 128:(kb + 1) * 128, :] = jnp.exp2(s - m).astype(BF)
                    mh.append(m)
                ms.append(mh)
            for hh in range(HG):
                ols = []
                for kb in range(3):
                    ols.append(_dot(vT_scr[g, B + kb, hh], eT_scr[t * HG + hh, kb * 128:(kb + 1) * 128, :]))
                m0 = jnp.where(B >= 2, ms[hh][0], NEG)
                m1 = jnp.where(B >= 1, ms[hh][1], NEG)
                m2 = ms[hh][2]
                mm = jnp.maximum(jnp.maximum(m0, m1), m2)
                c0 = jnp.where(B >= 2, jnp.exp2(m0 - mm), 0.0)
                c1 = jnp.where(B >= 1, jnp.exp2(m1 - mm), 0.0)
                c2 = jnp.exp2(m2 - mm)
                l = c0 * ols[0][DH:DH + 1] + c1 * ols[1][DH:DH + 1] + c2 * ols[2][DH:DH + 1]
                rl = 1.0 / l
                f0 = c0 * rl
                f1 = c1 * rl
                f2 = c2 * rl
                oT = ols[0][:DH] * f0 + ols[1][:DH] * f1 + ols[2][:DH] * f2
                oT_scr[b, pl.ds(pl.multiple_of(g * 128 + hh * DH, DH), DH), :] = oT
                f_scr[t * HG + hh, 0:1, :] = f0
                f_scr[t * HG + hh, 1:2, :] = f1
                f_scr[t * HG + hh, 2:3, :] = f2
            return carry

        lax.fori_loop(0, 2 * NG, fwd_body, 0)

        @pl.when(i == 0)
        def _wait_w():
            for k in range(1, 5):
                w_copy(k).wait()

        oT = jnp.concatenate([oT_scr[0], oT_scr[1]], axis=1)
        o = oT.T
        o_b = o.astype(BF)
        h = x + _dot(o_b, wo_ref[...])
        hn, r2 = _ln(h)
        hn_b = hn.astype(BF)
        gt = _dot_nt(hn_b, wg_ref[...])
        up = _dot_nt(hn_b, wu_ref[...])
        sg = jax.nn.sigmoid(gt)
        a_b = (sg * up).astype(BF)
        out = h + _dot(a_b, wd_ref[...])
        out_ref[...] = out.astype(out_ref.dtype)

        dout_b = dout_ref[...]
        dout = dout_b.astype(F32)
        da = _dot_nt(dout_b, wd_ref[...])
        a_wd[...] += _dot_tn(a_b, dout_b)
        du_b = (da * sg).astype(BF)
        dg_b = (da * up * sg * (1.0 - sg)).astype(BF)
        a_wg[...] += _dot_tn(dg_b, hn_b)
        a_wu[...] += _dot_tn(du_b, hn_b)
        dhn = _dot(dg_b, wg_ref[...]) + _dot(du_b, wu_ref[...])
        dh = dout + _ln_bwd(dhn, hn, r2)
        dh_scr[slot] = dh
        dh_b = dh.astype(BF)
        a_wo[...] += _dot_tn(o_b, dh_b)
        do = _dot_nt(dh_b, wo_ref[...])
        for g in range(NG):
            do_scr[g] = do[:, g * 128:(g + 1) * 128].astype(BF)
        doT = do.T
        doT_scr[0] = doT[:, 0:128]
        doT_scr[1] = doT[:, 128:256]
        prod = doT * oT
        dl = jnp.sum(prod.reshape(H, DH, TM), axis=1)
        dl_scr[0] = dl[:, 0:128]
        dl_scr[1] = dl[:, 128:256]

        @pl.when(i == NB - 1)
        def _flush_mlp():
            o_wd[...] = a_wd[...].astype(BF)
            g_copy(4).start()
            o_wg[...] = a_wg[...].astype(BF)
            g_copy(2).start()
            o_wu[...] = a_wu[...].astype(BF)
            g_copy(3).start()
            o_wo[...] = a_wo[...].astype(BF)
            g_copy(1).start()

        def bwd_body(t, carry):
            b = t // NG
            g = t % NG
            B = 2 * i + b
            dog = do_scr[g, pl.ds(pl.multiple_of(b * QB, QB), QB), :]
            di = pltpu.bitcast(dog, jnp.int32)
            for hh in range(HG):
                bd_scr[hh * 128:(hh + 1) * 128, :] = pltpu.bitcast(
                    jnp.where(lane64 // DH == hh, di, jnp.zeros_like(di)), BF)
            vwin = vn_scr[g, pl.ds(pl.multiple_of(B * 128, 128), KW), :]
            s_scr[...] = _dot_nt(vwin, bd_scr[...])
            for hh in range(HG):
                delta = dl_scr[b, pl.ds(g * HG + hh, 1), :]
                for kb in range(3):
                    dp = s_scr[kb * 128:(kb + 1) * 128, hh * 128:(hh + 1) * 128]
                    e = eT_scr[t * HG + hh, kb * 128:(kb + 1) * 128, :]
                    f = f_scr[t * HG + hh, kb:kb + 1, :]
                    ds_scr[hh, kb * 128:(kb + 1) * 128, :] = (e.astype(F32) * ((dp - delta) * f)).astype(BF)
            for hh in range(HG):
                hrow = pl.multiple_of(g * 128 + hh * DH, DH)
                doT_h = doT_scr[b, pl.ds(hrow, DH), :]
                qT_h = qT_scr[b, pl.ds(hrow, DH), :]
                dqT = None
                for kb in range(3):
                    e = eT_scr[t * HG + hh, kb * 128:(kb + 1) * 128, :]
                    ds = ds_scr[hh, kb * 128:(kb + 1) * 128, :]
                    f = f_scr[t * HG + hh, kb:kb + 1, :]
                    cv = _dot_nt((doT_h * f).astype(BF), e)
                    ck = _dot_nt(qT_h, ds)
                    if kb == 2:
                        dvT_acc[g, B + kb, hh * DH:(hh + 1) * DH, :] = cv
                        dkT_acc[g, B + kb, hh * DH:(hh + 1) * DH, :] = ck
                    else:
                        dvT_acc[g, B + kb, hh * DH:(hh + 1) * DH, :] += cv
                        dkT_acc[g, B + kb, hh * DH:(hh + 1) * DH, :] += ck
                    c = _dot(kT_scr[g, B + kb, hh * DH:(hh + 1) * DH, :], ds)
                    dqT = c if dqT is None else dqT + c
                dqT_scr[slot, b, pl.ds(hrow, DH), :] = dqT * SCALE
            return carry

        lax.fori_loop(0, 2 * NG, bwd_body, 0)

    @pl.when(i > 0)
    def _lag():
        j = i - 1
        slot = j % 2
        xl = xl_ref[...].astype(F32)
        xn, r1 = _ln(xl)
        xnT_b = xn.T.astype(BF)
        cols = []
        for b in range(2):
            parts = [dqT_scr[slot, b].astype(BF)]
            for g in range(NG):
                parts.append((dkT_acc[g, 2 + 2 * j + b] * (1.0 / LOG2E)).astype(BF))
            for g in range(NG):
                parts.append(dvT_acc[g, 2 + 2 * j + b].astype(BF))
            cols.append(jnp.concatenate(parts, axis=0))
        dqkvT_b = jnp.concatenate(cols, axis=1)
        a_wqkv[...] += _dot_nt(xnT_b, dqkvT_b)

        @pl.when(i == NB)
        def _flush_qkv():
            o_wqkv[...] = a_wqkv[...].astype(BF)
            g_copy(0).start()

        dxn = _dot(wqkv_ref[...], dqkvT_b).T
        dx = dh_scr[slot] + _ln_bwd(dxn, xn, r1)
        dx_ref[...] = dx.astype(dx_ref.dtype)

    @pl.when(i == NB)
    def _fin():
        for k in (4, 2, 3, 1, 0):
            g_copy(k).wait()


@jax.jit
def pallas_sequential_preLN__sliding_block__glu_gated_glu__prompt_kernel(
    A_x: jax.Array,
    A_wqkv: jax.Array,
    A_wo: jax.Array,
    B_x: jax.Array,
    B_w_gate: jax.Array,
    B_w_up: jax.Array,
    B_w_down: jax.Array,
    grad_out: jax.Array,
):
    x2 = A_x.reshape(S, D)
    go = grad_out.reshape(S, D)

    cur = lambda i: (jnp.minimum(i, NB - 1), 0)
    lag = lambda i: (jnp.maximum(i - 1, 0), 0)
    const = lambda i: (0, 0)

    out_shape = (
        jax.ShapeDtypeStruct((S, D), BF),
        jax.ShapeDtypeStruct((S, D), BF),
        jax.ShapeDtypeStruct((D, 3 * D), BF),
        jax.ShapeDtypeStruct((D, D), BF),
        jax.ShapeDtypeStruct((F, D), BF),
        jax.ShapeDtypeStruct((F, D), BF),
        jax.ShapeDtypeStruct((F, D), BF),
    )
    in_specs = [
        pl.BlockSpec((TM, D), cur),
        pl.BlockSpec((TM, D), lag),
        pl.BlockSpec((TM, D), cur),
        pl.BlockSpec(memory_space=pl.ANY),
        pl.BlockSpec(memory_space=pl.ANY),
        pl.BlockSpec(memory_space=pl.ANY),
        pl.BlockSpec(memory_space=pl.ANY),
        pl.BlockSpec(memory_space=pl.ANY),
    ]
    out_specs = (
        pl.BlockSpec((TM, D), cur),
        pl.BlockSpec((TM, D), lag),
        pl.BlockSpec(memory_space=pl.ANY),
        pl.BlockSpec(memory_space=pl.ANY),
        pl.BlockSpec(memory_space=pl.ANY),
        pl.BlockSpec(memory_space=pl.ANY),
        pl.BlockSpec(memory_space=pl.ANY),
    )
    scratch = [
        pltpu.VMEM((NG, TM, 128), BF),
        pltpu.VMEM((2, D, QB), BF),
        pltpu.VMEM((NG, PAD + S, 128), BF),
        pltpu.VMEM((NG, PAD + S, 128), BF),
        pltpu.VMEM((NG, NKB, 128, 128), BF),
        pltpu.VMEM((NG, NKB, HG, 32, 128), BF),
        pltpu.VMEM((2 * H, KW, QB), BF),
        pltpu.VMEM((2 * H, 8, QB), F32),
        pltpu.VMEM((2, D, QB), F32),
        pltpu.VMEM((NG, TM, 128), BF),
        pltpu.VMEM((2, D, QB), F32),
        pltpu.VMEM((2, H, QB), F32),
        pltpu.VMEM((2, 2, D, QB), F32),
        pltpu.VMEM((NG, NKB, 128, 128), F32),
        pltpu.VMEM((NG, NKB, 128, 128), F32),
        pltpu.VMEM((2, TM, D), F32),
        pltpu.VMEM((D, 3 * D), F32),
        pltpu.VMEM((D, D), F32),
        pltpu.VMEM((F, D), F32),
        pltpu.VMEM((F, D), F32),
        pltpu.VMEM((F, D), F32),
        pltpu.VMEM((HG * 128, 128), BF),
        pltpu.VMEM((KW, HG * 128), F32),
        pltpu.VMEM((HG, KW, 128), BF),
        pltpu.VMEM((D, 3 * D), BF),
        pltpu.VMEM((D, D), BF),
        pltpu.VMEM((F, D), BF),
        pltpu.VMEM((F, D), BF),
        pltpu.VMEM((F, D), BF),
        pltpu.VMEM((D, 3 * D), BF),
        pltpu.VMEM((D, D), BF),
        pltpu.VMEM((F, D), BF),
        pltpu.VMEM((F, D), BF),
        pltpu.VMEM((F, D), BF),
        pltpu.SemaphoreType.DMA((10,)),
    ]
    outs = pl.pallas_call(
        _kernel,
        grid=(NB + 1,),
        in_specs=in_specs,
        out_specs=out_specs,
        out_shape=out_shape,
        scratch_shapes=scratch,
        compiler_params=pltpu.CompilerParams(
            dimension_semantics=("arbitrary",),
            vmem_limit_bytes=100 * 1024 * 1024,
        ),
    )(x2, x2, go, A_wqkv, A_wo, B_w_gate.T, B_w_up.T, B_w_down)
    fwd, dx, dwqkv, dwo, dwg, dwu, dwd = outs
    return (fwd.reshape(1, S, D), dx.reshape(1, S, D), dwqkv, dwo, dwg.T, dwu.T, dwd)
```
